```python
import jax
import jax.numpy as jnp

def _softmax(x, axis=-1):
    return jax.nn.softmax(x, axis=axis)
def _gelu(x):
    return jax.nn.gelu(x, approximate=True)
def _silu(x):
    return jax.nn.silu(x)
def _sigmoid(x):
    return jax.nn.sigmoid(x)
def _layernorm(x, axis=-1, eps=1e-5):
    m = jnp.mean(x, axis=axis, keepdims=True)
    v = jnp.var(x, axis=axis, keepdims=True)
    return (x - m) / jnp.sqrt(v + eps)
def _scatter_add(tgt, idx, src, axis=0):
    return tgt.at[idx].add(src)
def _segment_sum(src, seg, n):
    return jax.ops.segment_sum(src, seg, n)
class _Rng:
    def __init__(self, key):
        self._k = key
    def _next(self):
        self._k, sub = jax.random.split(self._k)
        return sub
    def normal(self, shape):
        return jax.random.normal(self._next(), shape, dtype=jnp.bfloat16)
    def randint(self, lo, hi, shape):
        return jax.random.randint(self._next(), shape, lo, hi, dtype=jnp.int32)
    def uniform(self, shape, lo=0.0, hi=1.0):
        return jax.random.uniform(self._next(), shape, jnp.bfloat16, lo, hi)
    def permutation(self, n):
        return jax.random.permutation(self._next(), n)


kernel_name = 'interleave_layers__sliding_local_dilated__dense_activation_gelu__prompt'

def setup_inputs():
    _rng = _Rng(jax.random.key(int.from_bytes(__import__("os").urandom(4), "little")))
    _w = (lambda a: (lambda t: t.astype(jnp.bfloat16) if jnp.issubdtype(t.dtype, jnp.floating) else t)(jnp.asarray(a)))
    def _A_setup():
        B, S, D = 1, 2048, 1024
        return {
            "x": _w((lambda *s: _rng.normal(s) * 0.05)(B, S, D)),
            "wqkv": _w((lambda *s: _rng.normal(s) * 0.05)(D, 3 * D)),
            "wo": _w((lambda *s: _rng.normal(s) * 0.05)(D, D)),
        }
    _A_in = _A_setup()

    def _B_setup():
        B, S, D, F = 1, 2048, 1024, 3584
        return {
            "x": _w((lambda *s: _rng.normal(s) * 0.05)(B, S, D)),
            "w1": _w((lambda *s: _rng.normal(s) * 0.05)(D, F) * (D ** -0.5)),
            "b1": _w((lambda *s: _rng.normal(s) * 0.05)(F) * 0.01),
            "w2": _w((lambda *s: _rng.normal(s) * 0.05)(F, D) * (F ** -0.5)),
            "b2": _w((lambda *s: _rng.normal(s) * 0.05)(D) * 0.01),
        }
    _B_in = _B_setup()

    return {
        "A_x": _A_in["x"],
        "A_wqkv": _A_in["wqkv"],
        "A_wo": _A_in["wo"],
        "B_x": _B_in["x"],
        "B_w1": _B_in["w1"],
        "B_b1": _B_in["b1"],
        "B_w2": _B_in["w2"],
        "B_b2": _B_in["b2"],
    }

def reference(A_x, A_wqkv, A_wo, B_x, B_w1, B_b1, B_w2, B_b2):
    def _A_ref(x, wqkv, wo):
        B, S, D = x.shape
        H = 32; Dh = D // H
        W, dil = 8, 2
        qkv = (lambda x, *d: x.transpose(*d))((x @ wqkv).reshape(B, S, 3, H, Dh), 2, 0, 3, 1, 4)
        q, k, v = qkv[0], qkv[1], qkv[2]
        scale = Dh ** -0.5
        pos = jnp.arange(S)
        off = jnp.arange(W) * dil
        idx = pos[:, None] - off[None, :]
        mask = idx >= 0
        idx_c = jnp.where(mask, idx, 0).reshape(-1)
        kg = k[:, :, idx_c, :].reshape(B, H, S, W, Dh)
        vg = v[:, :, idx_c, :].reshape(B, H, S, W, Dh)
        logits = jnp.einsum("bhsd,bhswd->bhsw", q, kg) * scale
        logits = jnp.where(mask[None, None, :, :], logits, -1e9)
        attn = _softmax(logits, axis=-1)
        o = jnp.einsum("bhsw,bhswd->bhsd", attn, vg)
        return (lambda x, *d: x.transpose(*d))(o, 0, 2, 1, 3).reshape(B, S, D) @ wo

    def _B_ref(x, w1, b1, w2, b2):
        h = jnp.einsum("bsd,df->bsf", x, w1) + b1
        h = _gelu(h)
        return jnp.einsum("bsf,fd->bsd", h, w2) + b2

    x = A_x
    x = x + _A_ref(_layernorm(x, axis=-1), A_wqkv, A_wo)
    x = x + _B_ref(_layernorm(x, axis=-1), B_w1, B_b1, B_w2, B_b2)
    x = x + _A_ref(_layernorm(x, axis=-1), A_wqkv, A_wo)
    x = x + _B_ref(_layernorm(x, axis=-1), B_w1, B_b1, B_w2, B_b2)
    return x
```

```python
import functools, math
import jax
import jax.numpy as jnp
import jax.experimental.pallas as pl
import jax.experimental.pallas.tpu as pltpu

S, D, F, H, DH, W, DIL = 2048, 1024, 3584, 32, 32, 8, 2
T = 256
C = T // 8
HALO = (W - 1) * DIL
NJ = D // 128
FC = 512
EPS = 1e-5
F32, BF16 = jnp.float32, jnp.bfloat16
EXP2_SCALE = (DH ** -0.5) * math.log2(math.e)


def _ln(x):
    m = jnp.mean(x, axis=-1, keepdims=True)
    xc = x - m
    v = jnp.mean(xc * xc, axis=-1, keepdims=True)
    return xc * jax.lax.rsqrt(v + EPS)


def _gelu(x):
    c = math.sqrt(2.0 / math.pi)
    u = x * (c + (c * 0.044715) * (x * x))
    hx = 0.5 * x
    return hx + hx * jnp.tanh(u)


def _attn_group(q_s, k_s, v_s, b, G, first_tile):
    R = 8 * G
    r0 = 8 * b
    qs = [q_s[r0:r0 + R, j * 128:(j + 1) * 128] for j in range(NJ)]
    ss = []
    for w in range(W):
        k0 = r0 + 8 * (HALO - DIL * w)
        s = qs[0] * k_s[k0:k0 + R, 0:128]
        for j in range(1, NJ):
            s = s + qs[j] * k_s[k0:k0 + R, j * 128:(j + 1) * 128]
        s = s + pltpu.roll(s, 64, 1)
        s = s + pltpu.roll(s, 32, 1)
        if b < DIL * w:
            row = jax.lax.broadcasted_iota(jnp.int32, (R, 128), 0)
            bad = ((row & 7) == 0) & ((row >> 3) + (b - DIL * w) < 0) & first_tile
            s = jnp.where(bad, -1e9, s)
        ss.append(s)
    m = ss[0]
    for w in range(1, W):
        m = jnp.maximum(m, ss[w])
    es = [jnp.exp2((s - m) * EXP2_SCALE) for s in ss]
    den = es[0]
    for w in range(1, W):
        den = den + es[w]
    inv = 1.0 / den
    ps = [e * inv for e in es]
    outs = []
    for j in range(NJ):
        k0 = r0 + 8 * HALO
        o = ps[0] * v_s[k0:k0 + R, j * 128:(j + 1) * 128]
        for w in range(1, W):
            k0 = r0 + 8 * (HALO - DIL * w)
            o = o + ps[w] * v_s[k0:k0 + R, j * 128:(j + 1) * 128]
        outs.append(o)
    return outs


def kernel(x_ref, wqkv_ref, wo_ref, w1_ref, b1_ref, w2_ref, b2_ref, o_ref,
           xs, tmp, q_s, k_s, v_s, o_s, hk, hv):
    i = pl.program_id(0)
    l = pl.program_id(1)

    @pl.when(l == 0)
    def _():
        for j in range(NJ):
            tmp[j] = x_ref[:, j * 128:(j + 1) * 128].astype(F32)
        for b in range(C):
            for j in range(NJ):
                xs[8 * b:8 * b + 8, j * 128:(j + 1) * 128] = tmp[j, pl.ds(b, 8, stride=C), :]

    @pl.when(i == 0)
    def _():
        hk[l] = jnp.zeros(hk.shape[1:], F32)
        hv[l] = jnp.zeros(hv.shape[1:], F32)

    h = _ln(xs[...]).astype(BF16)
    q_s[...] = jnp.dot(h, wqkv_ref[:, 0:D], preferred_element_type=F32)
    k_s[8 * HALO:, :] = jnp.dot(h, wqkv_ref[:, D:2 * D], preferred_element_type=F32)
    v_s[8 * HALO:, :] = jnp.dot(h, wqkv_ref[:, 2 * D:3 * D], preferred_element_type=F32)
    sub0 = jax.lax.broadcasted_iota(jnp.int32, (8, D), 0) == 0
    for src, hal in ((k_s, hk), (v_s, hv)):
        for b in range(HALO):
            cur = pltpu.roll(src[T + 8 * b:T + 8 * b + 8, :], 1, 0)
            src[8 * b:8 * b + 8, :] = jnp.where(sub0, hal[l, 8 * b:8 * b + 8, :], cur)
            hal[l, 8 * b:8 * b + 8, :] = cur
    G = 2
    first = i == 0
    for b in range(0, C, G):
        outs = _attn_group(q_s, k_s, v_s, b, G, first)
        for j in range(NJ):
            o_s[8 * b:8 * (b + G), j * 128:(j + 1) * 128] = outs[j].astype(BF16)
    x1 = xs[...] + jnp.dot(o_s[...], wo_ref[...], preferred_element_type=F32)
    h2 = _ln(x1).astype(BF16)
    acc = x1 + b2_ref[...].astype(F32)
    for f in range(0, F, FC):
        u = jnp.dot(h2, w1_ref[:, f:f + FC], preferred_element_type=F32) + b1_ref[:, f:f + FC].astype(F32)
        g = _gelu(u).astype(BF16)
        acc = acc + jnp.dot(g, w2_ref[f:f + FC, :], preferred_element_type=F32)
    xs[...] = acc

    @pl.when(l == 1)
    def _():
        for b in range(C):
            for j in range(NJ):
                tmp[j, pl.ds(b, 8, stride=C), :] = xs[8 * b:8 * b + 8, j * 128:(j + 1) * 128]
        for j in range(NJ):
            o_ref[:, j * 128:(j + 1) * 128] = tmp[j].astype(BF16)


@jax.jit
def pallas_interleave_layers__sliding_local_dilated__dense_activation_gelu__prompt_kernel(
        A_x, A_wqkv, A_wo, B_x, B_w1, B_b1, B_w2, B_b2):
    x = A_x.reshape(S, D)
    wqkv = A_wqkv.reshape(D, 3, H, DH).transpose(0, 1, 3, 2).reshape(D, 3 * D)
    wo = A_wo.reshape(H, DH, D).transpose(1, 0, 2).reshape(D, D)
    const = lambda shape: pl.BlockSpec(shape, lambda i, l: (0, 0), pipeline_mode=pl.Buffered(1))
    out = pl.pallas_call(
        kernel,
        grid=(S // T, 2),
        in_specs=[pl.BlockSpec((T, D), lambda i, l: (i, 0)),
                  const((D, 3 * D)), const((D, D)), const((D, F)), const((1, F)),
                  const((F, D)), const((1, D))],
        out_specs=pl.BlockSpec((T, D), lambda i, l: (i, 0)),
        out_shape=jax.ShapeDtypeStruct((S, D), BF16),
        scratch_shapes=[pltpu.VMEM((T, D), F32), pltpu.VMEM((NJ, T, 128), F32), pltpu.VMEM((T, D), F32),
                        pltpu.VMEM((T + 8 * HALO, D), F32), pltpu.VMEM((T + 8 * HALO, D), F32),
                        pltpu.VMEM((T, D), BF16),
                        pltpu.VMEM((2, 8 * HALO, D), F32), pltpu.VMEM((2, 8 * HALO, D), F32)],
        compiler_params=pltpu.CompilerParams(dimension_semantics=("arbitrary", "arbitrary"),
                                             vmem_limit_bytes=100 * 1024 * 1024),
    )(x, wqkv, wo, B_w1, B_b1.reshape(1, F), B_w2, B_b2.reshape(1, D))
    return out.reshape(1, S, D)
```

```python
import math
import jax
import jax.numpy as jnp
import jax.experimental.pallas as pl
import jax.experimental.pallas.tpu as pltpu

S, D, F, H, DH, W, DIL = 2048, 1024, 3584, 32, 32, 8, 2
T = 256
NT = S // T
NI = 2 * NT
SKEW = 4
C = T // 8
HALO = (W - 1) * DIL
NJ = D // 128
MH, KH = T // 2, D // 2
MQ, DQ, FQ = T // 4, D // 4, F // 4
PITCH = 40
NP1, NP2 = 30, 8
EPS = 1e-5
F32, BF16, U32 = jnp.float32, jnp.bfloat16, jnp.uint32
EXP2_SCALE = (DH ** -0.5) * math.log2(math.e)


def _quad(g):
    n = len(g) // 2
    return ([r[:n] for r in g[:n]], [r[n:] for r in g[:n]],
            [r[:n] for r in g[n:]], [r[n:] for r in g[n:]])


def _add(a, b):
    return [[x + y for x, y in zip(ra, rb)] for ra, rb in zip(a, b)]


def _sub(a, b):
    return [[x - y for x, y in zip(ra, rb)] for ra, rb in zip(a, b)]


def _lhs_variants(g):
    if len(g) == 1:
        yield g[0][0]
        return
    a11, a12, a21, a22 = _quad(g)
    yield from _lhs_variants(a11)
    yield from _lhs_variants(_add(a11, a12))
    yield from _lhs_variants(_add(a11, a22))
    yield from _lhs_variants(_sub(a12, a22))
    yield from _lhs_variants(a22)
    yield from _lhs_variants(_add(a21, a22))
    yield from _lhs_variants(_sub(a21, a11))


def _rhs_variants(g):
    if len(g) == 1:
        yield g[0][0]
        return
    b11, b12, b21, b22 = _quad(g)
    yield from _rhs_variants(_sub(b12, b22))
    yield from _rhs_variants(b22)
    yield from _rhs_variants(_add(b11, b22))
    yield from _rhs_variants(_add(b21, b22))
    yield from _rhs_variants(_sub(b21, b11))
    yield from _rhs_variants(b11)
    yield from _rhs_variants(_add(b11, b12))


def _combine(prod, level, base=0, emit=lambda r, c, blocks: None):
    if level == 0:
        r = yield from prod(base)
        return [[r]]
    n = 7 ** (level - 1)
    m3 = yield from _combine(prod, level - 1, base)
    m5 = yield from _combine(prod, level - 1, base + n)
    c12 = _add(m3, m5)
    emit(0, 1, c12)
    m1 = yield from _combine(prod, level - 1, base + 2 * n)
    c11 = _sub(m1, m5)
    c22 = _add(m1, m3)
    c11 = _add(c11, (yield from _combine(prod, level - 1, base + 3 * n)))
    m4 = yield from _combine(prod, level - 1, base + 4 * n)
    c11 = _add(c11, m4)
    emit(0, 0, c11)
    m2 = yield from _combine(prod, level - 1, base + 5 * n)
    c21 = _add(m2, m4)
    emit(1, 0, c21)
    c22 = _sub(c22, m2)
    c22 = _add(c22, (yield from _combine(prod, level - 1, base + 6 * n)))
    emit(1, 1, c22)
    return [a + b for a, b in zip(c11, c12)] + [a + b for a, b in zip(c21, c22)]


def _unpack(x32, e):
    return pltpu.unpack_elementwise(x32, index=e, packed_dtype=BF16, unpacked_dtype=F32)


def _rhs_packed(even, odd):
    for a, b in zip(_rhs_variants(even), _rhs_variants(odd)):
        yield pltpu.pack_elementwise([a, b], packed_dtype=BF16)


def _mm(a, b32):
    return jnp.dot(a, pltpu.bitcast(b32, BF16), preferred_element_type=F32)


def _interleave(*streams):
    streams = [s for s in streams if s is not None]
    done = [0] * len(streams)
    alive = [True] * len(streams)
    while any(alive):
        i = min((j for j in range(len(streams)) if alive[j]), key=lambda j: done[j] / streams[j][1])
        try:
            next(streams[i][0])
            done[i] += 1
        except StopIteration:
            alive[i] = False


def _take(gen, n):
    for _ in range(n):
        next(gen)
        yield


def _chain(*gens):
    for gen in gens:
        yield from gen


def _run(gen):
    for _ in gen:
        pass


def _gelu(x):
    c = math.sqrt(2.0 / math.pi)
    u = x * (c + (c * 0.044715) * (x * x))
    hx = 0.5 * x
    return hx + hx * jnp.tanh(u)


def _ln_rows(xs, slot, r0, n):
    blk = [xs[slot, j, r0:r0 + n, :] for j in range(NJ)]
    s = blk[0]
    for b in blk[1:]:
        s = s + b
    m = jnp.sum(s, axis=-1, keepdims=True) * (1.0 / D)
    cs = [b - m for b in blk]
    q = cs[0] * cs[0]
    for c in cs[1:]:
        q = q + c * c
    r = jax.lax.rsqrt(jnp.sum(q, axis=-1, keepdims=True) * (1.0 / D) + EPS)
    return [c * r for c in cs]


def _split(load, level):
    n = 2 ** level
    return [[load(r * T // n, T // n, c * D // n, D // n) for c in range(n)] for r in range(n)]


class _Lazy:
    def __init__(self, grid):
        self.gen = _lhs_variants(grid)
        self.vals = []

    def __getitem__(self, n):
        while len(self.vals) <= n:
            self.vals.append(next(self.gen).astype(BF16))
        return self.vals[n]


def _kernel(x_hbm, wqkv_hbm, wo_hbm, w1_hbm, b1_ref, w2_hbm, b2_ref, o_hbm,
            xb, xs, h2_s, o_s, p_s, q_s, k_s, v_s, hk, hvv, t_s, to_s,
            wqkv_r, wo_r, w1_r, w2_r, wqkv_v, wo_v, w1_v, w2_v, sems):
    full = (q_s, k_s, v_s, o_s, p_s)
    lds = [None]
    q_s, k_s, v_s, o_s, p_s = q_s.at[0], k_s.at[0], v_s.at[0], o_s.at[0], p_s.at[0]
    h_s = p_s.at[T + 8:2 * T + 8]
    R1, R2 = DQ // SKEW, FQ // SKEW
    KV = T + 8 * HALO

    def qkv_copy(p, rc, hf):
        r = hf * KH + rc * 128
        return pltpu.make_async_copy(wqkv_hbm.at[pl.ds(r, 128), pl.ds(p * D, D)],
                                     wqkv_r.at[p, pl.ds(r, 128), :], sems.at[(p * 4 + rc) * 2 + hf])

    def in_copy(t):
        return pltpu.make_async_copy(x_hbm.at[pl.ds(t * T, T), :], xb.at[t], sems.at[25 + 8 * SKEW + t])

    def out_copy(t):
        return pltpu.make_async_copy(xb.at[t], o_hbm.at[pl.ds(t * T, T), :], sems.at[25 + 8 * SKEW + NT + t])

    def wo_copy():
        return pltpu.make_async_copy(wo_hbm, wo_r, sems.at[24])

    def mlp_copies(c):
        out = []
        for q in range(4):
            r = q * DQ + c * R1
            out.append(pltpu.make_async_copy(w1_hbm.at[pl.ds(r, R1), :], w1_r.at[pl.ds(r, R1), :],
                                             sems.at[25 + c * 8 + q]))
            r = q * FQ + c * R2
            out.append(pltpu.make_async_copy(w2_hbm.at[pl.ds(r, R2), :], w2_r.at[pl.ds(r, R2), :],
                                             sems.at[25 + c * 8 + 4 + q]))
        return out

    last = [None]

    def mm(a, b32):
        last[0] = _mm(a, b32)
        return last[0]

    def gate(ref, *idx):
        if last[0] is not None:
            n = 16 if ref.dtype == BF16 else 8
            ref[idx[:-1] + (slice(idx[-1], idx[-1] + n), slice(0, 128))] = last[0][0:n, 0:128].astype(ref.dtype)

    def x_in(t, slot):
        for a in range(8):
            for j in range(NJ):
                xs[slot, j, pl.ds(a, C, stride=8), :] = xb[t, a * C:(a + 1) * C, j * 128:(j + 1) * 128].astype(F32)
                if j % 2:
                    yield

    def x_out(slot):
        for a in range(8):
            for j in range(NJ):
                if j % 4 == 0:
                    gate(xs, NT, 0, 0)
                xb[slot, a * C:(a + 1) * C, j * 128:(j + 1) * 128] = xs[slot, j, pl.ds(a, C, stride=8), :].astype(BF16)
                if j % 4 == 3:
                    yield

    def ln(slot, dst, n, lag=0, extra=None):
        pend = []
        for r in range(0, T + lag * n, n):
            if r < T:
                gate(xs, NT, 0, 0)
                pend.append((r, _ln_rows(xs, slot, r, n)))
                if extra is not None:
                    next(extra)
            if r >= lag * n:
                r0, vals = pend.pop(0)
                for j, v in enumerate(vals):
                    dst[r0:r0 + n, j * 128:(j + 1) * 128] = v
            yield

    def prep_mlp(c):
        for raw, dst, kq, nq, rows in ((w1_r, w1_v, DQ, FQ, R1), (w2_r, w2_v, FQ, DQ, R2)):
            for r in range(0, rows, 16):
                r0 = pl.multiple_of(c * rows + r, 16)
                d0 = pl.multiple_of(c * (rows // 2) + r // 2, 8)
                for cb in range(nq // 128):
                    gate(raw, 4 * kq)
                    blk = [[pltpu.bitcast(raw[pl.ds(rq * kq + r0, 16), cq * nq + cb * 128:cq * nq + (cb + 1) * 128], U32)
                            for cq in range(4)] for rq in range(4)]
                    ev, od = ([[_unpack(b, e) for b in row] for row in blk] for e in range(2))
                    for i, v in enumerate(_rhs_packed(ev, od)):
                        dst[i, pl.ds(d0, 8), cb * 128:(cb + 1) * 128] = v
                    yield

    def startup():
        in_copy(0).start()
        for p in range(3):
            for rc in range(4):
                qkv_copy(p, rc, 0).start()
                qkv_copy(p, rc, 1).start()
        in_copy(1).start()
        wo_copy().start()
        for c in range(SKEW):
            in_copy(2 + c).start()
            for cp in mlp_copies(c):
                cp.start()
        for t in range(2 + SKEW, NT):
            in_copy(t).start()
        hk[...] = jnp.zeros(hk.shape, F32)
        hvv[...] = jnp.zeros(hvv.shape, F32)
        in_copy(0).wait()
        _run(x_in(0, 0))
        _run(ln(0, h_s, 16))

        def prep_qkv(it, carry):
            p, rc = it // 4, it % 4
            qkv_copy(p, rc, 0).wait()
            qkv_copy(p, rc, 1).wait()
            r0 = pl.multiple_of(rc * 128, 128)
            top = pltpu.bitcast(wqkv_r[p, pl.ds(r0, 128), :], U32)
            bot = pltpu.bitcast(wqkv_r[p, pl.ds(KH + r0, 128), :], U32)
            wt = jnp.concatenate([top, bot], axis=0).T
            for h in range(H):
                t_s[h * PITCH:h * PITCH + DH, :] = wt[h * DH:(h + 1) * DH, :]
            d0 = pl.multiple_of(rc * 64, 64)
            for jj in range(NJ // 2):
                cols = [jnp.concatenate([t_s[pl.ds(4 * j + dd, H, stride=PITCH), :] for dd in range(4)], axis=0).T
                        for j in (jj, jj + NJ // 2)]
                ev, od = ([[_unpack(c[hf * 64:(hf + 1) * 64], e) for c in cols] for hf in range(2)]
                          for e in range(2))
                for i, v in enumerate(_rhs_packed(ev, od)):
                    wqkv_v[p * 7 + i, pl.ds(d0, 64), jj * 128:(jj + 1) * 128] = v
            return carry

        jax.lax.fori_loop(0, 12, prep_qkv, 0)
        in_copy(1).wait()
        _run(x_in(1, 1))
        wo_copy().wait()
        for j in range(NJ):
            for h in range(H):
                to_s[j, h % 2, (h // 2) * 24:(h // 2) * 24 + 16, :] = pltpu.bitcast(
                    wo_r[h * DH:(h + 1) * DH, j * 128:(j + 1) * 128], U32)
        for jj in range(NJ // 2):
            for dp in range(8):
                raw = [[[to_s[j, par, pl.ds(dq, 16, stride=24), :] for j in (jj, jj + NJ // 2)]
                        for dq in (dp, dp + 8)] for par in range(2)]
                for e in range(2):
                    ev, od = ([[_unpack(b, e) for b in row] for row in raw[par]] for par in range(2))
                    d = 2 * dp + e
                    for i, v in enumerate(_rhs_packed(ev, od)):
                        wo_v[i, d * 16:(d + 1) * 16, jj * 128:(jj + 1) * 128] = v

    def wide(a, w, n, nt):
        out = []
        for t in range(nt):
            out.append(mm(a, w[n, :, t * 128:(t + 1) * 128]))
            yield
        return jnp.concatenate(out, axis=1) if nt > 1 else out[0]

    def halo(src, srl, hal, lay, b):
        sub0 = jax.lax.broadcasted_iota(jnp.int32, (8, D), 0) == 0
        cur = pltpu.roll(srl[T + 8 * b:T + 8 * b + 8, :], 1, 0)
        src[8 * b:8 * b + 8, :] = jnp.where(sub0, hal[lay, 8 * b:8 * b + 8, :], cur)
        hal[lay, 8 * b:8 * b + 8, :] = cur

    def y_qkv():
        hv = _Lazy(_split(lambda r, nr, c, nc: h_s[r:r + nr, c:c + nc], 1))
        for p, (dst, off) in enumerate(((q_s, 0), (k_s, 8 * HALO), (v_s, 8 * HALO))):
            def emit(r, c, blk):
                dst[off + r * MH:off + (r + 1) * MH, c * KH:(c + 1) * KH] = blk[0][0]
            yield from _combine(lambda n: wide(hv[n], wqkv_v, p * 7 + n, 4), 1, emit=emit)
            yield

    order = list(range(HALO, C)) + list(range(HALO))

    def y_probs(k):
        q_l, k_l = lds[0][:2]
        first = (k % NT) == 0
        row0 = jax.lax.broadcasted_iota(jnp.int32, (8, 128), 0) == 0
        for i, b in enumerate(order):
            ss = []
            for w in range(W):
                if w % 4 == 0:
                    gate(k_s, KV)
                    if w == 0 and i < HALO:
                        halo(k_s, k_l, hk, k // NT, i)
                    qs = [q_l[8 * b:8 * b + 8, j * 128:(j + 1) * 128] for j in range(NJ)]
                k0 = 8 * (b + HALO - DIL * w)
                s = qs[0] * k_l[k0:k0 + 8, 0:128]
                for j in range(1, NJ):
                    s = s + qs[j] * k_l[k0:k0 + 8, j * 128:(j + 1) * 128]
                s = s + pltpu.roll(s, 64, 1)
                s = s + pltpu.roll(s, 32, 1)
                if b < DIL * w:
                    s = jnp.where(row0 & first, -1e9, s)
                ss.append(s)
                if w == 3:
                    yield
            m = ss[0]
            for w in range(1, W):
                m = jnp.maximum(m, ss[w])
            es = [jnp.exp2((s - m) * EXP2_SCALE) for s in ss]
            den = es[0]
            for w in range(1, W):
                den = den + es[w]
            inv = 1.0 / den
            for w in range(W):
                p_s[8 * b:8 * b + 8, w * 128:(w + 1) * 128] = es[w] * inv
            yield

    def y_pv(k):
        v_l, p_l = lds[0][2], lds[0][4]
        for i, b in enumerate(order):
            for j in range(NJ):
                if j % 4 == 0:
                    gate(p_s, T)
                    if j == 0 and i < HALO:
                        gate(v_s, KV)
                        halo(v_s, v_l, hvv, k // NT, i)
                    ps = [p_l[8 * b:8 * b + 8, w * 128:(w + 1) * 128] for w in range(W)]
                o = None
                for w in range(W):
                    k0 = 8 * (b + HALO - DIL * w)
                    t = ps[w] * v_l[k0:k0 + 8, j * 128:(j + 1) * 128]
                    o = t if o is None else o + t
                o_s[8 * b:8 * b + 8, j * 128:(j + 1) * 128] = o
                if j % 4 == 3:
                    yield

    def y_wo(slot):
        o_l = lds[0][3]
        ov = _Lazy(_split(lambda r, nr, c, nc: o_l[r:r + nr, c:c + nc], 1))

        def emit(r, c, blk):
            for jj in range(NJ // 2):
                xs[slot, c * (NJ // 2) + jj, r * MH:(r + 1) * MH, :] += blk[0][0][:, jj * 128:(jj + 1) * 128]
        yield from _combine(lambda n: wide(ov[n], wo_v, n, 4), 1, emit=emit)

    gl = []

    def m_w1():
        h2 = _Lazy(_split(lambda r, nr, c, nc: h2_s[r:r + nr, c:c + nc], 2))
        for f in range(0, FQ, 128):
            u = yield from _combine(lambda n: wide(h2[n], w1_v.at[:, :, f:f + 128], n, 1), 2)
            gl.append([[_gelu(u[r][c] + b1_ref[:, c * FQ + f:c * FQ + f + 128].astype(F32)) for c in range(4)]
                       for r in range(4)])

    def m_w2(slot):
        gv = _Lazy([[jnp.concatenate([ch[r][c] for ch in gl], axis=1) for c in range(4)] for r in range(4)])

        def emit(r, c, blk):
            for rr in range(2):
                for jj in range(NJ // 2):
                    j, r0 = c * (NJ // 2) + jj, (2 * r + rr) * MQ
                    xs[slot, j, r0:r0 + MQ, :] += (blk[rr][jj // 2][:, (jj % 2) * 128:(jj % 2 + 1) * 128]
                                                  + b2_ref[:, j * 128:(j + 1) * 128].astype(F32))
        yield from _combine(lambda n: wide(gv[n], w2_v, n, 2), 2, emit=emit)

    def step(g, do_y, do_m):
        z = g >> 20
        lds[0] = [r.at[z] for r in full]
        last[0] = None
        del gl[:]
        k = g
        s = g - SKEW
        ky, kn, sm = k % NT, (k + 1) % NT, s % NT
        x_slot = jnp.where(k + 2 < NT, k + 2, NT)
        x_t = jnp.minimum(k + 2, NT - 1)
        if do_m and do_y:
            qkv, w1, pr = y_qkv(), m_w1(), y_probs(k)
            _interleave((_take(qkv, 20), 20), (ln(sm, h2_s, 16), 16))
            _interleave((_take(qkv, 38), 38), (_take(w1, 98), 98))
            _interleave((_take(qkv, 16), 16), (w1, 245), (_take(pr, NP1), NP1))
            _interleave((qkv, 13), (_take(pr, NP2), NP2))
            _interleave((m_w2(sm), 98), (_chain(pr, y_pv(k)), 130 - NP1 - NP2),
                        (ln(kn, h_s, 8, 2, x_in(x_t, x_slot)), 36))
            _interleave((y_wo(ky), 28), (x_out(sm), 18))
        elif do_m:
            _run(ln(sm, h2_s, 16))
            _run(m_w1())
            _run(m_w2(sm))
            last[0] = None
            _run(x_out(sm))
        else:
            qkv = y_qkv()
            _interleave((_take(qkv, 58), 58), (prep_mlp(g), 57))
            _interleave((qkv, 29), (y_probs(k), 64))
            last[0] = None
            _run(y_pv(k))
            _interleave((y_wo(ky), 28), (ln(kn, h_s, 8, 0, x_in(x_t, x_slot)), 33))

    def p_step(g, carry):
        in_copy(g + 2).wait()
        for cp in mlp_copies(g):
            cp.wait()
        step(g, True, False)
        return carry

    def s_step(g, carry):
        step(g, True, True)

        @pl.when(g >= SKEW + NT)
        def _():
            out_copy(g - SKEW - NT).start()
        return carry

    def e_step(g, carry):
        step(g, False, True)
        out_copy(g - SKEW - NT).start()
        return carry

    startup()
    jax.lax.fori_loop(0, SKEW, p_step, 0)
    for t in range(2 + SKEW, NT):
        in_copy(t).wait()
    jax.lax.fori_loop(SKEW, NI, s_step, 0)
    jax.lax.fori_loop(NI, NI + SKEW, e_step, 0)
    for t in range(NT):
        out_copy(t).wait()


@jax.jit
def pallas_interleave_layers__sliding_local_dilated__dense_activation_gelu__prompt_kernel(
        A_x, A_wqkv, A_wo, B_x, B_w1, B_b1, B_w2, B_b2):
    x = A_x.reshape(S, D)
    hbm = pl.BlockSpec(memory_space=pl.ANY)
    vm = pltpu.VMEM
    out = pl.pallas_call(
        _kernel,
        in_specs=[hbm, hbm, hbm, hbm, pl.BlockSpec(memory_space=vm), hbm, pl.BlockSpec(memory_space=vm)],
        out_specs=hbm,
        out_shape=jax.ShapeDtypeStruct((S, D), BF16),
        scratch_shapes=[
            vm((NT, T, D), BF16),
            vm((NT + 1, NJ, T, 128), F32),
            vm((T, D), F32),
            vm((1, T, D), F32), vm((1, 2 * T + 8, D), F32),
            vm((1, T, D), F32), vm((1, T + 8 * HALO + 8, D), F32), vm((1, T + 8 * HALO + 8, D), F32),
            vm((2, 8 * HALO, D), F32), vm((2, 8 * HALO, D), F32),
            vm((H * PITCH, 128), U32), vm((NJ, 2, 16 * 24, 128), U32),
            vm((3, D, D), BF16), vm((D, D), BF16), vm((D + 16, F), BF16), vm((F + 16, D), BF16),
            vm((21, KH // 2, KH), U32), vm((7, KH // 2, KH), U32),
            vm((49, DQ // 2, FQ), U32), vm((49, FQ // 2, DQ), U32),
            pltpu.SemaphoreType.DMA((25 + 8 * SKEW + 2 * NT,)),
        ],
        compiler_params=pltpu.CompilerParams(vmem_limit_bytes=127 * 1024 * 1024),
    )(x, A_wqkv, A_wo, B_w1, B_b1.reshape(1, F), B_w2, B_b2.reshape(1, D))
    return out.reshape(1, S, D)
```

```python
import math
import jax
import jax.numpy as jnp
import jax.experimental.pallas as pl
import jax.experimental.pallas.tpu as pltpu

S, D, F, H, DH, W, DIL = 2048, 1024, 3584, 32, 32, 8, 2
T = 256
NT = S // T
NI = 2 * NT
SKEW = 3
NCH = SKEW - 1
C = T // 8
HALO = (W - 1) * DIL
NJ = D // 128
MH, KH = T // 2, D // 2
MQ, DQ, FQ = T // 4, D // 4, F // 4
PITCH = 40
NP1, NP2 = 24, 8
LAGW = 4
NVH = 52
NW1, NW2 = 60, 75
EPS = 1e-5
F32, BF16, U32 = jnp.float32, jnp.bfloat16, jnp.uint32
EXP2_SCALE = (DH ** -0.5) * math.log2(math.e)


def _quad(g):
    n = len(g) // 2
    return ([r[:n] for r in g[:n]], [r[n:] for r in g[:n]],
            [r[:n] for r in g[n:]], [r[n:] for r in g[n:]])


def _add(a, b):
    return [[x + y for x, y in zip(ra, rb)] for ra, rb in zip(a, b)]


def _sub(a, b):
    return [[x - y for x, y in zip(ra, rb)] for ra, rb in zip(a, b)]


def _lhs_variants(g):
    if len(g) == 1:
        yield g[0][0]
        return
    a11, a12, a21, a22 = _quad(g)
    yield from _lhs_variants(a11)
    yield from _lhs_variants(_add(a11, a12))
    yield from _lhs_variants(_add(a11, a22))
    yield from _lhs_variants(_sub(a12, a22))
    yield from _lhs_variants(a22)
    yield from _lhs_variants(_add(a21, a22))
    yield from _lhs_variants(_sub(a21, a11))


def _rhs_variants(g):
    if len(g) == 1:
        yield g[0][0]
        return
    b11, b12, b21, b22 = _quad(g)
    yield from _rhs_variants(_sub(b12, b22))
    yield from _rhs_variants(b22)
    yield from _rhs_variants(_add(b11, b22))
    yield from _rhs_variants(_add(b21, b22))
    yield from _rhs_variants(_sub(b21, b11))
    yield from _rhs_variants(b11)
    yield from _rhs_variants(_add(b11, b12))


def _combine(prod, level, base=0, emit=lambda r, c, blocks: None):
    if level == 0:
        r = yield from prod(base)
        return [[r]]
    n = 7 ** (level - 1)
    m3 = yield from _combine(prod, level - 1, base)
    m5 = yield from _combine(prod, level - 1, base + n)
    c12 = _add(m3, m5)
    emit(0, 1, c12)
    m1 = yield from _combine(prod, level - 1, base + 2 * n)
    c11 = _sub(m1, m5)
    c22 = _add(m1, m3)
    c11 = _add(c11, (yield from _combine(prod, level - 1, base + 3 * n)))
    m4 = yield from _combine(prod, level - 1, base + 4 * n)
    c11 = _add(c11, m4)
    emit(0, 0, c11)
    m2 = yield from _combine(prod, level - 1, base + 5 * n)
    c21 = _add(m2, m4)
    emit(1, 0, c21)
    c22 = _sub(c22, m2)
    c22 = _add(c22, (yield from _combine(prod, level - 1, base + 6 * n)))
    emit(1, 1, c22)
    return [a + b for a, b in zip(c11, c12)] + [a + b for a, b in zip(c21, c22)]


def _unpack(x32, e):
    return pltpu.unpack_elementwise(x32, index=e, packed_dtype=BF16, unpacked_dtype=F32)


def _rhs_packed(even, odd):
    for a, b in zip(_rhs_variants(even), _rhs_variants(odd)):
        yield pltpu.pack_elementwise([a, b], packed_dtype=BF16)


def _mm(a, b32):
    return jnp.dot(a, pltpu.bitcast(b32, BF16), preferred_element_type=F32)


def _interleave(*streams):
    streams = [s for s in streams if s is not None]
    done = [0] * len(streams)
    alive = [True] * len(streams)
    while any(alive):
        i = min((j for j in range(len(streams)) if alive[j]), key=lambda j: done[j] / streams[j][1])
        try:
            next(streams[i][0])
            done[i] += 1
        except StopIteration:
            alive[i] = False


def _take(gen, n):
    for _ in range(n):
        next(gen)
        yield


def _chain(*gens):
    for gen in gens:
        yield from gen


def _run(gen):
    for _ in gen:
        pass


def _gelu2(x):
    c = math.sqrt(2.0 / math.pi)
    u = x * (c + (c * 0.044715) * (x * x))
    return x + x * jnp.tanh(u)


def _ln_rows(xs, slot, r0, n):
    blk = [xs[slot, j, r0:r0 + n, :] for j in range(NJ)]
    s = blk[0]
    for b in blk[1:]:
        s = s + b
    m = jnp.sum(s, axis=-1, keepdims=True) * (1.0 / D)
    cs = [b - m for b in blk]
    q = cs[0] * cs[0]
    for c in cs[1:]:
        q = q + c * c
    r = jax.lax.rsqrt(jnp.sum(q, axis=-1, keepdims=True) * (1.0 / D) + EPS)
    return [c * r for c in cs]


def _split(load, level):
    n = 2 ** level
    return [[load(r * T // n, T // n, c * D // n, D // n) for c in range(n)] for r in range(n)]


class _Lazy:
    def __init__(self, grid, gen=None):
        self.gen = gen or _lhs_variants(grid)
        self.vals = []

    def __getitem__(self, n):
        while len(self.vals) <= n:
            self.vals.append(next(self.gen).astype(BF16))
        return self.vals[n]


def _kernel(x_hbm, wqkv_hbm, wo_hbm, w1_hbm, b1_ref, w2_hbm, b2_ref, o_hbm,
            xb, xs, h2_s, q_s, k_s, v_s, hk, hvv, t_s, to_s,
            wqkv_r, wo_r, w1_r, w2_r, wqkv_v, wo_v, w1_v, w2_v, sems):
    full = (q_s, k_s, v_s, h2_s)
    lds = [None]
    q_s, k_s, v_s = q_s.at[0], k_s.at[0], v_s.at[0]
    h2_s = h2_s.at[0]
    hn_s = q_s.at[T + 8:2 * T + 8]
    h_s = xs.at[NT + 1]
    R1, R2 = DQ // NCH, FQ // NCH
    KV = T + 8 * HALO

    def qkv_copy(p, rc, hf):
        r = hf * KH + rc * 128
        return pltpu.make_async_copy(wqkv_hbm.at[pl.ds(r, 128), pl.ds(p * D, D)],
                                     wqkv_r.at[p, pl.ds(r, 128), :], sems.at[(p * 4 + rc) * 2 + hf])

    def in_copy(t):
        return pltpu.make_async_copy(x_hbm.at[pl.ds(t * T, T), :], xb.at[t], sems.at[25 + 8 * NCH + t])

    def out_copy(t):
        return pltpu.make_async_copy(xb.at[t], o_hbm.at[pl.ds(t * T, T), :], sems.at[25 + 8 * NCH + NT + t])

    def wo_copy():
        return pltpu.make_async_copy(wo_hbm, wo_r.at[0, pl.ds(0, D), :], sems.at[24])

    def mlp_copies(c):
        out = []
        for q in range(4):
            r = q * DQ + c * R1
            out.append(pltpu.make_async_copy(w1_hbm.at[pl.ds(r, R1), :], w1_r.at[pl.ds(r, R1), :],
                                             sems.at[25 + c * 8 + q]))
            r = q * FQ + c * R2
            out.append(pltpu.make_async_copy(w2_hbm.at[pl.ds(r, R2), :], w2_r.at[pl.ds(r, R2), :],
                                             sems.at[25 + c * 8 + 4 + q]))
        return out

    last = [None, 0]

    def mm(a, b32):
        last[0], last[1] = _mm(a, b32), 0
        return last[0]

    def gate(ref, *idx, adv=0):
        if last[0] is not None:
            n = 16 if ref.dtype == BF16 else 8
            r = min(last[1], last[0].shape[0] - n)
            last[1] += adv
            ref[idx[:-1] + (slice(idx[-1], idx[-1] + n), slice(0, 128))] = (
                pltpu.bitcast(last[0][r:r + n, 0:128], U32) if ref.dtype == U32 else last[0][r:r + n, 0:128].astype(ref.dtype))

    def x_in(t, slot):
        for a in range(8):
            for j in range(NJ):
                xs[slot, j, pl.ds(a, C, stride=8), :] = xb[t, a * C:(a + 1) * C, j * 128:(j + 1) * 128].astype(F32)
                if j % 2:
                    yield

    def x_out(slot):
        for a in range(8):
            for j in range(NJ):
                if j % 4 == 0:
                    gate(xs, NT, 0, 0)
                xb[slot, a * C:(a + 1) * C, j * 128:(j + 1) * 128] = xs[slot, j, pl.ds(a, C, stride=8), :].astype(BF16)
                if j % 4 == 3:
                    yield

    def ln(slot, dst, n, lag=0, extra=None):
        pend = []
        for r in range(0, T + lag * n, n):
            if r < T:
                gate(xs, NT, 0, 0)
                pend.append((r, _ln_rows(xs, slot, r, n)))
                if extra is not None:
                    next(extra)
            if r >= lag * n:
                r0, vals = pend.pop(0)
                for j, v in enumerate(vals):
                    if dst is h_s:
                        dst[j, r0:r0 + n, :] = v
                        if lag and j == 0 and r0 >= T - lag * n:
                            q_s[T:T + 8, 0:128] = v[0:8]
                    else:
                        dst[r0:r0 + n, j * 128:(j + 1) * 128] = v
            yield

    def prep_mlp(c):
        for raw, dst, kq, nq, rows, half in ((w1_r, w1_v, DQ, FQ, R1, 0), (w2_r, w2_v, FQ, DQ, R2, 1)):
            for r in range(0, rows, 16):
                r0 = pl.multiple_of(c * rows + r, 16)
                d0 = pl.multiple_of(c * (rows // 2) + r // 2, 8)
                for cb in range(nq // 128):
                    def quad(qr, qc):
                        gate(raw, 4 * kq, adv=16)
                        blk = [[pltpu.bitcast(raw[pl.ds(rq * kq + r0, 16), pl.ds(cq * nq + cb * 128, 128)], U32)
                                for cq in (qc, qc + 1)] for rq in (qr, qr + 1)]
                        return [[[_unpack(b, e) * 0.5 if half else _unpack(b, e) for b in row] for row in blk]
                                for e in range(2)]

                    def put(i, grids):
                        for n, v in enumerate(_rhs_packed(*grids)):
                            dst[7 * i + n, pl.ds(d0, 8), cb * 128:(cb + 1) * 128] = v

                    b22 = quad(2, 2)
                    put(1, b22)
                    for i, op, q in ((0, _sub, (0, 2)), (2, _add, (0, 0)), (3, _add, (2, 0))):
                        yield
                        put(i, map(op, quad(*q), b22))
                    yield
                    b11 = quad(0, 0)
                    put(5, b11)
                    for i, op, q in ((4, _sub, (2, 0)), (6, _add, (0, 2))):
                        yield
                        put(i, map(op, quad(*q), b11))
                    yield

    def wide(a, w, n, nt, bias=None):
        out = []
        for t in range(nt):
            out.append(mm(a, w[n, :, t * 128:(t + 1) * 128]))
            if bias is not None and n // 7 in (0, 4) and n % 7 in (0, 4):
                out[-1] = out[-1] + bias(2 * (n // 7 == 0) + (n % 7 == 0), t).astype(F32)
            yield
        return jnp.concatenate(out, axis=1) if nt > 1 else out[0]

    def halo(src, srl, hal, lay, b):
        sub0 = jax.lax.broadcasted_iota(jnp.int32, (8, D), 0) == 0
        cur = pltpu.roll(srl[T + 8 * b:T + 8 * b + 8, :], 1, 0)
        src[8 * b:8 * b + 8, :] = jnp.where(sub0, hal[lay, 8 * b:8 * b + 8, :], cur)
        hal[lay, 8 * b:8 * b + 8, :] = cur

    def y_qkv(by_tile=False):
        hv = _Lazy(_split(lambda r, nr, c, nc: jnp.concatenate(
            [h_s[j, r:r + nr, :] for j in range(c // 128, (c + nc) // 128)], axis=1), 1))
        for p, (dst, off) in enumerate(((q_s, 0), (k_s, 8 * HALO), (v_s, 8 * HALO))):
            if by_tile:
                for t in range(0, KH, 128):
                    def emit(r, c, blk):
                        dst[off + r * MH:off + (r + 1) * MH, c * KH + t:c * KH + t + 128] = blk[0][0]
                    yield from _combine(lambda n: wide(hv[n], wqkv_v.at[:, :, t:t + 128], p * 7 + n, 1), 1, emit=emit)
                continue

            def emit(r, c, blk):
                dst[off + r * MH:off + (r + 1) * MH, c * KH:(c + 1) * KH] = blk[0][0]
            yield from _combine(lambda n: wide(hv[n], wqkv_v, p * 7 + n, 4), 1, emit=emit)
            yield

    order = list(range(HALO, C)) + list(range(HALO))

    def flush(pend, dst=q_s, keep=0):
        while len(pend) > keep:
            b, j, v = pend.pop(0)
            dst[8 * b:8 * b + 8, j * 128:(j + 1) * 128] = v

    def y_probs(k, loose=False):
        q_l, k_l = lds[0][:2]
        dst = h2_s if loose else q_s
        first = jnp.asarray((k % NT) == 0)
        row0 = jax.lax.broadcasted_iota(jnp.int32, (8, 128), 0) == 0
        pend = []
        for i, b in enumerate(order):
            ss = []
            for w in range(W):
                if w % 4 == 0:
                    gate(k_s, KV)
                    if w == 0 and i < HALO:
                        halo(k_s, k_l, hk, k // NT, i)
                    qs = [q_l[8 * b:8 * b + 8, j * 128:(j + 1) * 128] for j in range(NJ)]
                    if w == LAGW:
                        flush(pend, dst, W)
                k0 = 8 * (b + HALO - DIL * w)
                s = qs[0] * k_l[k0:k0 + 8, 0:128]
                for j in range(1, NJ):
                    s = s + qs[j] * k_l[k0:k0 + 8, j * 128:(j + 1) * 128]
                s = s + pltpu.roll(s, 64, 1)
                s = s + pltpu.roll(s, 32, 1)
                if b < DIL * w:
                    s = jnp.where(row0 & first, -1e9, s)
                ss.append(s)
                if w == 3:
                    yield
            m = ss[0]
            for w in range(1, W):
                m = jnp.maximum(m, ss[w])
            es = [jnp.exp2((s - m) * EXP2_SCALE) for s in ss]
            den = es[0]
            for w in range(1, W):
                den = den + es[w]
            inv = 1.0 / den
            pend += [(b, w, es[w] * inv) for w in range(W)]
            if i == C - 1:
                flush(pend, dst)
            yield

    def v_halo(k):
        for i in range(HALO):
            gate(v_s, KV)
            halo(v_s, lds[0][2], hvv, k // NT, i)
            yield

    def y_pv(k, loose=False):
        v_l, p_l = lds[0][2], lds[0][3 if loose else 0]
        pend = []
        halves = [(i, b, j0) for i, b in enumerate(order) for j0 in (0, 4)]
        if loose:
            _run(v_halo(k))
            halves = [(C, b, j0) for b0, j0 in ((0, 0), (0, 4), (16, 4), (16, 0)) for b in range(b0, b0 + 16)]
        for n, (i, b, j0) in enumerate(halves):
            for j in range(j0, j0 + 4):
                if j % 4 == 0:
                    gate(h2_s if loose else q_s, T, adv=32 if loose else 0)
                    ps = [p_l[8 * b:8 * b + 8, w * 128:(w + 1) * 128] for w in range(W)]
                    flush(pend)
                o = None
                for w in range(W):
                    k0 = 8 * (b + HALO - DIL * w)
                    t = ps[w] * v_l[k0:k0 + 8, j * 128:(j + 1) * 128]
                    o = t if o is None else o + t
                pend.append((b, j, o))
                if j % 4 == 3 and (loose or n == 2 * C - 1):
                    flush(pend)
                if j % 4 == 3:
                    yield

    upd = []

    def spread(gen, drain=True):
        for _ in gen:
            if upd:
                idx, v = upd.pop(0)
                xs[idx] += v
            yield
        while drain and upd:
            idx, v = upd.pop(0)
            xs[idx] += v

    def y_wo(slot):
        def variants():
            ld = lambda r, c: lds[0][0][r * MH:(r + 1) * MH, c * KH:(c + 1) * KH]
            a11 = ld(0, 0)
            yield a11
            a12 = ld(0, 1)
            yield a11 + a12
            a22 = ld(1, 1)
            yield a11 + a22
            yield a12 - a22
            yield a22
            a21 = ld(1, 0)
            yield a21 + a22
            yield a21 - a11
        ov = _Lazy(None, variants())

        def emit(r, c, blk):
            for jj in range(NJ // 2):
                upd.append(((slot, c * (NJ // 2) + jj, pl.ds(r * MH, MH)), blk[0][0][:, jj * 128:(jj + 1) * 128]))
        yield from spread(_combine(lambda n: wide(ov[n], wo_v, n, 4), 1, emit=emit))

    gl = []

    def m_w1():
        h2 = _Lazy(_split(lambda r, nr, c, nc: hn_s[r:r + nr, c:c + nc], 2))
        for f in range(0, FQ, 128):
            u = yield from _combine(lambda n: wide(h2[n], w1_v.at[:, :, f:f + 128], n, 1,
                                                   lambda c, t: b1_ref[:, c * FQ + f:c * FQ + f + 128]), 2)
            gl.append([[_gelu2(u[r][c]) for c in range(4)] for r in range(4)])

    def m_w2(slot, drain=True):
        gv = _Lazy([[jnp.concatenate([ch[r][c] for ch in gl], axis=1) for c in range(4)] for r in range(4)])

        def emit(r, c, blk):
            for rr in range(2):
                for jj in range(NJ // 2):
                    j, r0 = c * (NJ // 2) + jj, (2 * r + rr) * MQ
                    upd.append(((slot, j, pl.ds(r0, MQ)), blk[rr][jj // 2][:, (jj % 2) * 128:(jj % 2 + 1) * 128]))
        yield from spread(_combine(
            lambda n: wide(gv[n], w2_v, n, 2, lambda c, t: b2_ref[:, pl.ds(c * DQ + t * 128, 128)]), 2, emit=emit), drain)

    def step(g, do_y, do_m):
        z = g >> 20
        lds[0] = [r.at[z] for r in full]
        last[0] = None
        del gl[:]
        k = g
        s = g - SKEW
        ky, kn, sm = k % NT, (k + 1) % NT, s % NT
        if do_m and do_y:
            qkv, w1, pr = y_qkv(), m_w1(), y_probs(k)
            _interleave((_take(qkv, 29), 29), (_take(w1, NW1), NW1))
            _interleave((_take(qkv, 29), 29), (_take(w1, NW2), NW2), (ln(kn, h_s, 8, 2), 35))
            _interleave((_take(qkv, 16), 16), (w1, 343 - NW1 - NW2), (_take(pr, NP1), NP1))
            _interleave((qkv, 13), (_take(pr, NP2), NP2))
            _interleave((m_w2(sm), 98), (_chain(pr, y_pv(k)), 130 - NP1 - NP2),
                        (_chain(v_halo(k), ln((s + 1) % NT, hn_s, 8, 2)), NVH))
            _interleave((y_wo(ky), 28), (x_out(sm), 28))
        elif do_m:
            _run(m_w1())
            _interleave((m_w2(sm), 98), (_chain(x_out(sm - 1), ln(jnp.minimum(sm + 1, NT - 1), hn_s, 8)), 60))
        else:
            qkv = y_qkv()
            pm = prep_mlp(g - 1)
            _interleave((_take(qkv, 29), 29), (_take(pm, 300), 300))
            _interleave((_take(qkv, 29), 29), (_take(pm, 200), 200), (ln(kn, h_s, 8, 3, x_in(k + 2, k + 2)), 36))
            _interleave((qkv, 29), (y_probs(k, True), 64), (_take(pm, 100), 100))
            last[0] = None
            pv, wo = y_pv(k, True), y_wo(ky)
            _run(_take(pv, 16))
            _interleave((_take(wo, 4), 4), (_take(pv, 16), 16))
            _interleave((_take(wo, 4), 4), (_take(pv, 16), 16))
            _interleave((_take(wo, 12), 12), (pv, 17), (_take(pm, 104), 104))
            _interleave((wo, 8), (pm, 80))

    def prep_qkv(p, rc):
        qkv_copy(p, rc, 0).wait()
        qkv_copy(p, rc, 1).wait()
        r0 = rc * 128 if isinstance(rc, int) else pl.multiple_of(rc * 128, 128)
        top = pltpu.bitcast(wqkv_r[p, pl.ds(r0, 128), :], U32)
        bot = pltpu.bitcast(wqkv_r[p, pl.ds(KH + r0, 128), :], U32)
        wt = jnp.concatenate([top, bot], axis=0).T
        for h in range(H):
            t_s[h * PITCH:h * PITCH + DH, :] = wt[h * DH:(h + 1) * DH, :]
        d0 = rc * 64 if isinstance(rc, int) else pl.multiple_of(rc * 64, 64)
        for jj in range(NJ // 2):
            cols = [jnp.concatenate([t_s[pl.ds(4 * j + dd, H, stride=PITCH), :] for dd in range(4)], axis=0).T
                    for j in (jj, jj + NJ // 2)]
            ev, od = ([[_unpack(c[hf * 64:(hf + 1) * 64], e) for c in cols] for hf in range(2)]
                      for e in range(2))
            for i, v in enumerate(_rhs_packed(ev, od)):
                wqkv_v[p * 7 + i, pl.ds(d0, 64), jj * 128:(jj + 1) * 128] = v
            yield


    def prep_wo(z):
        for j in range(NJ):
            for h in range(H):
                if h % 8 == 0:
                    gate(wo_r, 0, D, adv=16)
                to_s[j, h % 2, (h // 2) * 24:(h // 2) * 24 + 16, :] = pltpu.bitcast(
                    wo_r[z, h * DH:(h + 1) * DH, j * 128:(j + 1) * 128], U32)
                if h % 8 == 7:
                    yield
        for jj in range(NJ // 2):
            for dp in range(8):
                for hh in range(2):
                    gate(to_s, 0, 0, 16, adv=16)
                    raw = [[[to_s[z + j, par, pl.ds(dq + hh * 8 * 24, 8, stride=24), :] for j in (jj, jj + NJ // 2)]
                            for dq in (dp, dp + 8)] for par in range(2)]
                    for e in range(2):
                        ev, od = ([[_unpack(b, e) for b in row] for row in raw[par]] for par in range(2))
                        for i, v in enumerate(_rhs_packed(ev, od)):
                            wo_v[i, pl.ds((2 * dp + e) * 16 + hh * 8, 8), jj * 128:(jj + 1) * 128] = v
                    yield

    def startup():
        in_copy(0).start()
        for p in range(3):
            if p == 2:
                in_copy(1).start()
            for rc in range(4):
                qkv_copy(p, rc, 0).start()
                qkv_copy(p, rc, 1).start()
        wo_copy().start()
        in_copy(2).start()
        for c in range(NCH):
            in_copy(3 + c).start()
            for cp in mlp_copies(c):
                cp.start()
        for t in range(3 + NCH, NT):
            in_copy(t).start()
        hk[...] = jnp.zeros(hk.shape, F32)
        hvv[...] = jnp.zeros(hvv.shape, F32)
        in_copy(0).wait()
        _run(x_in(0, 0))
        _run(ln(0, h_s, 16))


        def prep_q(rc, carry):
            _run(prep_qkv(0, rc))
            return rc >> 20

        z = jax.lax.fori_loop(0, 4, prep_q, 0)
        lds[0] = [r.at[z] for r in full]
        qkv = y_qkv(True)
        nxt = x_in(1, 1)
        for it in range(4, 12):
            if it == 8:
                in_copy(1).wait()
            _interleave((prep_qkv(it // 4, it % 4), 4), (_take(qkv, 7), 7), (_take(nxt, 8), 8) if it >= 8 else None)
        pr = y_probs(0, True)
        _interleave((_take(qkv, 10), 10), (_take(pr, 24), 24))
        wo_copy().wait()
        _interleave((qkv, 18), (pr, 40), (prep_wo(z), 100))
        in_copy(2).wait()
        last[0] = None
        pv, wo = y_pv(0, True), y_wo(0)
        _run(_take(pv, 16))
        _interleave((_take(wo, 4), 4), (_take(pv, 16), 16))
        _interleave((_take(wo, 4), 4), (_take(pv, 16), 16))
        _interleave((wo, 20), (pv, 30), (ln(z + 1, h_s, 8, 4, x_in(2, 2)), 38))

    def p_step(g, carry):
        in_copy(g + 2).wait()
        for cp in mlp_copies(g - 1):
            cp.wait()
        step(g, True, False)
        return carry

    def s_step(g, carry):
        step(g, True, True)

        @pl.when(jnp.logical_and(g >= SKEW + NT, g < NI - 1))
        def _():
            out_copy(g - SKEW - NT).start()
        return carry

    def e_step(g, carry):
        step(g, False, True)
        out_copy(g - SKEW - NT - 1).start()
        return carry

    startup()
    jax.lax.fori_loop(1, SKEW, p_step, 0)

    def load_x(t, carry):
        in_copy(t).wait()
        _run(x_in(t, t))
        return carry

    jax.lax.fori_loop(2 + SKEW, NT, load_x, 0)
    last[0] = None
    _run(ln(0, hn_s, 16))
    jax.lax.fori_loop(SKEW, NI, s_step, 0)
    jax.lax.fori_loop(NI, NI + SKEW, e_step, 0)
    last[0] = None
    _run(x_out(NT - 1))
    out_copy(NT - 1).start()
    for t in range(NT):
        out_copy(t).wait()


@jax.jit
def pallas_interleave_layers__sliding_local_dilated__dense_activation_gelu__prompt_kernel(
        A_x, A_wqkv, A_wo, B_x, B_w1, B_b1, B_w2, B_b2):
    x = A_x.reshape(S, D)
    hbm = pl.BlockSpec(memory_space=pl.ANY)
    vm = pltpu.VMEM
    out = pl.pallas_call(
        _kernel,
        in_specs=[hbm, hbm, hbm, hbm, pl.BlockSpec(memory_space=vm), hbm, pl.BlockSpec(memory_space=vm)],
        out_specs=hbm,
        out_shape=jax.ShapeDtypeStruct((S, D), BF16),
        scratch_shapes=[
            vm((NT, T, D), BF16),
            vm((NT + 2, NJ, T, 128), F32),
            vm((1, T + 8, D), F32),
            vm((1, 2 * T + 8, D), F32), vm((1, T + 8 * HALO + 8, D), F32), vm((1, T + 8 * HALO + 8, D), F32),
            vm((2, 8 * HALO, D), F32), vm((2, 8 * HALO, D), F32),
            vm((H * PITCH, 128), U32), vm((NJ, 2, 16 * 24, 128), U32),
            vm((3, D, D), BF16), vm((1, D + 16, D), BF16), vm((D + 16, F), BF16), vm((F + 16, D), BF16),
            vm((21, KH // 2, KH), U32), vm((7, KH // 2, KH), U32),
            vm((49, DQ // 2, FQ), U32), vm((49, FQ // 2, DQ), U32),
            pltpu.SemaphoreType.DMA((25 + 8 * NCH + 2 * NT,)),
        ],
        compiler_params=pltpu.CompilerParams(vmem_limit_bytes=127 * 1024 * 1024),
    )(x, A_wqkv, A_wo, B_w1, B_b1.reshape(1, F), B_w2, B_b2.reshape(1, D))
    return out.reshape(1, S, D)
```

```python
import math
import jax
import jax.numpy as jnp
import jax.experimental.pallas as pl
import jax.experimental.pallas.tpu as pltpu

S, D, F, H, DH, W, DIL = 2048, 1024, 3584, 32, 32, 8, 2
T = 256
NT = S // T
NI = 2 * NT
SKEW = 3
NCH = SKEW - 1
C = T // 8
HALO = (W - 1) * DIL
NJ = D // 128
MH, KH = T // 2, D // 2
MQ, DQ, FQ = T // 4, D // 4, F // 4
PITCH = 40
NP1, NP2 = 24, 8
LAGW = 4
NVH = 52
NW1, NW2 = 60, 75
EPS = 1e-5
F32, BF16, U32 = jnp.float32, jnp.bfloat16, jnp.uint32
EXP2_SCALE = (DH ** -0.5) * math.log2(math.e)


def _quad(g):
    n = len(g) // 2
    return ([r[:n] for r in g[:n]], [r[n:] for r in g[:n]],
            [r[:n] for r in g[n:]], [r[n:] for r in g[n:]])


def _add(a, b):
    return [[x + y for x, y in zip(ra, rb)] for ra, rb in zip(a, b)]


def _sub(a, b):
    return [[x - y for x, y in zip(ra, rb)] for ra, rb in zip(a, b)]


def _lhs_variants(g):
    if len(g) == 1:
        yield g[0][0]
        return
    a11, a12, a21, a22 = _quad(g)
    yield from _lhs_variants(a11)
    yield from _lhs_variants(_add(a11, a12))
    yield from _lhs_variants(_add(a11, a22))
    yield from _lhs_variants(_sub(a12, a22))
    yield from _lhs_variants(a22)
    yield from _lhs_variants(_add(a21, a22))
    yield from _lhs_variants(_sub(a21, a11))


def _rhs_variants(g):
    if len(g) == 1:
        yield g[0][0]
        return
    b11, b12, b21, b22 = _quad(g)
    yield from _rhs_variants(_sub(b12, b22))
    yield from _rhs_variants(b22)
    yield from _rhs_variants(_add(b11, b22))
    yield from _rhs_variants(_add(b21, b22))
    yield from _rhs_variants(_sub(b21, b11))
    yield from _rhs_variants(b11)
    yield from _rhs_variants(_add(b11, b12))


def _combine(prod, level, base=0, emit=lambda r, c, blocks: None):
    if level == 0:
        r = yield from prod(base)
        return [[r]]
    n = 7 ** (level - 1)
    m3 = yield from _combine(prod, level - 1, base)
    m5 = yield from _combine(prod, level - 1, base + n)
    c12 = _add(m3, m5)
    emit(0, 1, c12)
    m1 = yield from _combine(prod, level - 1, base + 2 * n)
    c11 = _sub(m1, m5)
    c22 = _add(m1, m3)
    c11 = _add(c11, (yield from _combine(prod, level - 1, base + 3 * n)))
    m4 = yield from _combine(prod, level - 1, base + 4 * n)
    c11 = _add(c11, m4)
    emit(0, 0, c11)
    m2 = yield from _combine(prod, level - 1, base + 5 * n)
    c21 = _add(m2, m4)
    emit(1, 0, c21)
    c22 = _sub(c22, m2)
    c22 = _add(c22, (yield from _combine(prod, level - 1, base + 6 * n)))
    emit(1, 1, c22)
    return [a + b for a, b in zip(c11, c12)] + [a + b for a, b in zip(c21, c22)]


def _unpack(x32, e):
    return pltpu.unpack_elementwise(x32, index=e, packed_dtype=BF16, unpacked_dtype=F32)


def _rhs_packed(even, odd):
    for a, b in zip(_rhs_variants(even), _rhs_variants(odd)):
        yield pltpu.pack_elementwise([a, b], packed_dtype=BF16)


def _mm(a, b32):
    return jnp.dot(a, pltpu.bitcast(b32, BF16), preferred_element_type=F32)


def _interleave(*streams):
    streams = [s for s in streams if s is not None]
    done = [0] * len(streams)
    alive = [True] * len(streams)
    while any(alive):
        i = min((j for j in range(len(streams)) if alive[j]), key=lambda j: done[j] / streams[j][1])
        try:
            next(streams[i][0])
            done[i] += 1
        except StopIteration:
            alive[i] = False


def _take(gen, n):
    for _ in range(n):
        next(gen)
        yield


def _chain(*gens):
    for gen in gens:
        yield from gen


def _run(gen):
    for _ in gen:
        pass


def _gelu2(x):
    c = math.sqrt(2.0 / math.pi)
    u = x * (c + (c * 0.044715) * (x * x))
    return x + x * jnp.tanh(u)


def _ln_rows(xs, slot, r0, n):
    blk = [xs[slot, j, r0:r0 + n, :] for j in range(NJ)]
    s = blk[0]
    for b in blk[1:]:
        s = s + b
    m = jnp.sum(s, axis=-1, keepdims=True) * (1.0 / D)
    cs = [b - m for b in blk]
    q = cs[0] * cs[0]
    for c in cs[1:]:
        q = q + c * c
    r = jax.lax.rsqrt(jnp.sum(q, axis=-1, keepdims=True) * (1.0 / D) + EPS)
    return [c * r for c in cs]


def _split(load, level):
    n = 2 ** level
    return [[load(r * T // n, T // n, c * D // n, D // n) for c in range(n)] for r in range(n)]


class _Lazy:
    def __init__(self, grid, gen=None):
        self.gen = gen or _lhs_variants(grid)
        self.vals = []

    def __getitem__(self, n):
        while len(self.vals) <= n:
            self.vals.append(next(self.gen).astype(BF16))
        return self.vals[n]


def _kernel(x_hbm, wqkv_hbm, wo_hbm, w1_hbm, b1_ref, w2_hbm, b2_ref, o_hbm,
            xb, xs, h2_s, q_s, k_s, v_s, hk, hvv, t_s, to_s,
            wqkv_r, wo_r, w1_r, w2_r, wqkv_v, wo_v, w1_v, w2_v, sems):
    full = (q_s, k_s, v_s, h2_s)
    lds = [None]
    q_s, k_s, v_s = q_s.at[0], k_s.at[0], v_s.at[0]
    h2_s = h2_s.at[0]
    hn_s = q_s.at[T + 8:2 * T + 8]
    h_s = xs.at[NT + 1]
    R1, R2 = DQ // NCH, FQ // NCH
    KV = T + 8 * HALO

    def qkv_copy(p, rc, hf):
        r = hf * KH + rc * 128
        return pltpu.make_async_copy(wqkv_hbm.at[pl.ds(r, 128), pl.ds(p * D, D)],
                                     wqkv_r.at[p, pl.ds(r, 128), :], sems.at[(p * 4 + rc) * 2 + hf])

    def in_copy(t):
        return pltpu.make_async_copy(x_hbm.at[pl.ds(t * T, T), :], xb.at[t], sems.at[25 + 8 * NCH + t])

    def out_copy(t):
        return pltpu.make_async_copy(xb.at[t], o_hbm.at[pl.ds(t * T, T), :], sems.at[25 + 8 * NCH + NT + t])

    def wo_copy():
        return pltpu.make_async_copy(wo_hbm, wo_r.at[0, pl.ds(0, D), :], sems.at[24])

    def mlp_copies(c):
        out = []
        for q in range(4):
            r = q * DQ + c * R1
            out.append(pltpu.make_async_copy(w1_hbm.at[pl.ds(r, R1), :], w1_r.at[pl.ds(r, R1), :],
                                             sems.at[25 + c * 8 + q]))
            r = q * FQ + c * R2
            out.append(pltpu.make_async_copy(w2_hbm.at[pl.ds(r, R2), :], w2_r.at[pl.ds(r, R2), :],
                                             sems.at[25 + c * 8 + 4 + q]))
        return out

    last = [None, 0]

    def mm(a, b32):
        last[0], last[1] = _mm(a, b32), 0
        return last[0]

    def gate(ref, *idx, adv=0):
        if last[0] is not None:
            n = 16 if ref.dtype == BF16 else 8
            r = min(last[1], last[0].shape[0] - n)
            last[1] += adv
            ref[idx[:-1] + (slice(idx[-1], idx[-1] + n), slice(0, 128))] = (
                pltpu.bitcast(last[0][r:r + n, 0:128], U32) if ref.dtype == U32 else last[0][r:r + n, 0:128].astype(ref.dtype))

    def x_in(t, slot):
        for a in range(8):
            for j in range(NJ):
                xs[slot, j, pl.ds(a, C, stride=8), :] = xb[t, a * C:(a + 1) * C, j * 128:(j + 1) * 128].astype(F32)
                if j % 2:
                    yield

    def x_out(slot):
        for a in range(8):
            for j in range(NJ):
                if j % 4 == 0:
                    gate(xs, NT, 0, 0)
                xb[slot, a * C:(a + 1) * C, j * 128:(j + 1) * 128] = xs[slot, j, pl.ds(a, C, stride=8), :].astype(BF16)
                if j % 4 == 3:
                    yield

    def ln(slot, dst, n, lag=0, extra=None):
        pend = []
        for r in range(0, T + lag * n, n):
            if r < T:
                gate(xs, NT, 0, 0)
                pend.append((r, _ln_rows(xs, slot, r, n)))
                if extra is not None:
                    next(extra)
            if r >= lag * n:
                r0, vals = pend.pop(0)
                for j, v in enumerate(vals):
                    if dst is h_s:
                        dst[j, r0:r0 + n, :] = v
                        if lag and j == 0 and r0 >= T - lag * n:
                            q_s[T:T + 8, 0:128] = v[0:8]
                    else:
                        dst[r0:r0 + n, j * 128:(j + 1) * 128] = v
            yield

    def prep_mlp(c):
        for raw, dst, kq, nq, rows, half in ((w1_r, w1_v, DQ, FQ, R1, 0), (w2_r, w2_v, FQ, DQ, R2, 1)):
            for r in range(0, rows, 16):
                r0 = pl.multiple_of(c * rows + r, 16)
                d0 = pl.multiple_of(c * (rows // 2) + r // 2, 8)
                for cb in range(nq // 128):
                    def quad(qr, qc):
                        gate(raw, 4 * kq, adv=16)
                        blk = [[pltpu.bitcast(raw[pl.ds(rq * kq + r0, 16), pl.ds(cq * nq + cb * 128, 128)], U32)
                                for cq in (qc, qc + 1)] for rq in (qr, qr + 1)]
                        return [[[_unpack(b, e) * 0.5 if half else _unpack(b, e) for b in row] for row in blk]
                                for e in range(2)]

                    def put(i, grids):
                        for n, v in enumerate(_rhs_packed(*grids)):
                            dst[7 * i + n, pl.ds(d0, 8), cb * 128:(cb + 1) * 128] = v

                    b22 = quad(2, 2)
                    put(1, b22)
                    for i, op, q in ((0, _sub, (0, 2)), (2, _add, (0, 0)), (3, _add, (2, 0))):
                        yield
                        put(i, map(op, quad(*q), b22))
                    yield
                    b11 = quad(0, 0)
                    put(5, b11)
                    for i, op, q in ((4, _sub, (2, 0)), (6, _add, (0, 2))):
                        yield
                        put(i, map(op, quad(*q), b11))
                    yield

    def wide(a, w, n, nt, bias=None):
        out = []
        for t in range(nt):
            out.append(mm(a, w[n, :, t * 128:(t + 1) * 128]))
            if bias is not None and n // 7 in (0, 4) and n % 7 in (0, 4):
                out[-1] = out[-1] + bias(2 * (n // 7 == 0) + (n % 7 == 0), t).astype(F32)
            yield
        return jnp.concatenate(out, axis=1) if nt > 1 else out[0]

    def halo(src, srl, hal, lay, b):
        sub0 = jax.lax.broadcasted_iota(jnp.int32, (8, D), 0) == 0
        cur = pltpu.roll(srl[T + 8 * b:T + 8 * b + 8, :], 1, 0)
        src[8 * b:8 * b + 8, :] = jnp.where(sub0, hal[lay, 8 * b:8 * b + 8, :], cur)
        hal[lay, 8 * b:8 * b + 8, :] = cur

    def y_qkv(by_tile=False):
        hv = _Lazy(_split(lambda r, nr, c, nc: jnp.concatenate(
            [h_s[j, r:r + nr, :] for j in range(c // 128, (c + nc) // 128)], axis=1), 1))
        for p, (dst, off) in enumerate(((q_s, 0), (k_s, 8 * HALO), (v_s, 8 * HALO))):
            if by_tile:
                for t in range(0, KH, 128):
                    def emit(r, c, blk):
                        dst[off + r * MH:off + (r + 1) * MH, c * KH + t:c * KH + t + 128] = blk[0][0]
                    yield from _combine(lambda n: wide(hv[n], wqkv_v.at[:, :, t:t + 128], p * 7 + n, 1), 1, emit=emit)
                continue

            def emit(r, c, blk):
                dst[off + r * MH:off + (r + 1) * MH, c * KH:(c + 1) * KH] = blk[0][0]
            yield from _combine(lambda n: wide(hv[n], wqkv_v, p * 7 + n, 4), 1, emit=emit)
            yield

    order = list(range(HALO, C)) + list(range(HALO))

    def flush(pend, dst=q_s, keep=0):
        while len(pend) > keep:
            b, j, v = pend.pop(0)
            dst[8 * b:8 * b + 8, j * 128:(j + 1) * 128] = v

    def y_probs(k, loose=False):
        q_l, k_l = lds[0][:2]
        dst = h2_s if loose else q_s
        first = jnp.asarray((k % NT) == 0)
        row0 = jax.lax.broadcasted_iota(jnp.int32, (8, 128), 0) == 0
        pend = []
        for i, b in enumerate(order):
            ss = []
            for w in range(W):
                if w % 4 == 0:
                    gate(k_s, KV)
                    if w == 0 and i < HALO:
                        halo(k_s, k_l, hk, k // NT, i)
                    qs = [q_l[8 * b:8 * b + 8, j * 128:(j + 1) * 128] for j in range(NJ)]
                    if w == LAGW:
                        flush(pend, dst, W)
                k0 = 8 * (b + HALO - DIL * w)
                s = qs[0] * k_l[k0:k0 + 8, 0:128]
                for j in range(1, NJ):
                    s = s + qs[j] * k_l[k0:k0 + 8, j * 128:(j + 1) * 128]
                s = s + pltpu.roll(s, 64, 1)
                s = s + pltpu.roll(s, 32, 1)
                if b < DIL * w:
                    s = jnp.where(row0 & first, -1e9, s)
                ss.append(s)
                if w == 3:
                    yield
            m = ss[0]
            for w in range(1, W):
                m = jnp.maximum(m, ss[w])
            es = [jnp.exp2((s - m) * EXP2_SCALE) for s in ss]
            den = es[0]
            for w in range(1, W):
                den = den + es[w]
            inv = 1.0 / den
            pend += [(b, w, es[w] * inv) for w in range(W)]
            if i == C - 1:
                flush(pend, dst)
            yield

    def v_halo(k):
        for i in range(HALO):
            gate(v_s, KV)
            halo(v_s, lds[0][2], hvv, k // NT, i)
            yield

    def y_pv(k, loose=False):
        v_l, p_l = lds[0][2], lds[0][3 if loose else 0]
        pend = []
        halves = [(i, b, j0) for i, b in enumerate(order) for j0 in (0, 4)]
        if loose:
            _run(v_halo(k))
            halves = [(C, b, j0) for b0, j0 in ((0, 0), (0, 4), (16, 4), (16, 0)) for b in range(b0, b0 + 16)]
        for n, (i, b, j0) in enumerate(halves):
            for j in range(j0, j0 + 4):
                if j % 4 == 0:
                    gate(h2_s if loose else q_s, T, adv=32 if loose else 0)
                    ps = [p_l[8 * b:8 * b + 8, w * 128:(w + 1) * 128] for w in range(W)]
                    flush(pend)
                o = None
                for w in range(W):
                    k0 = 8 * (b + HALO - DIL * w)
                    t = ps[w] * v_l[k0:k0 + 8, j * 128:(j + 1) * 128]
                    o = t if o is None else o + t
                pend.append((b, j, o))
                if j % 4 == 3 and (loose or n == 2 * C - 1):
                    flush(pend)
                if j % 4 == 3:
                    yield

    upd = []

    def spread(gen, drain=True):
        for _ in gen:
            if upd:
                idx, v = upd.pop(0)
                xs[idx] += v
            yield
        while drain and upd:
            idx, v = upd.pop(0)
            xs[idx] += v

    def y_wo(slot):
        def variants():
            ld = lambda r, c: lds[0][0][r * MH:(r + 1) * MH, c * KH:(c + 1) * KH]
            a11 = ld(0, 0)
            yield a11
            a12 = ld(0, 1)
            yield a11 + a12
            a22 = ld(1, 1)
            yield a11 + a22
            yield a12 - a22
            yield a22
            a21 = ld(1, 0)
            yield a21 + a22
            yield a21 - a11
        ov = _Lazy(None, variants())

        def emit(r, c, blk):
            for jj in range(NJ // 2):
                upd.append(((slot, c * (NJ // 2) + jj, pl.ds(r * MH, MH)), blk[0][0][:, jj * 128:(jj + 1) * 128]))
        yield from spread(_combine(lambda n: wide(ov[n], wo_v, n, 4), 1, emit=emit))

    gl = []

    def m_w1():
        h2 = _Lazy(_split(lambda r, nr, c, nc: hn_s[r:r + nr, c:c + nc], 2))
        for f in range(0, FQ, 128):
            u = yield from _combine(lambda n: wide(h2[n], w1_v.at[:, :, f:f + 128], n, 1,
                                                   lambda c, t: b1_ref[:, c * FQ + f:c * FQ + f + 128]), 2)
            gl.append([[_gelu2(u[r][c]) for c in range(4)] for r in range(4)])

    def m_w2(slot, drain=True):
        gv = _Lazy([[jnp.concatenate([ch[r][c] for ch in gl], axis=1) for c in range(4)] for r in range(4)])

        def emit(r, c, blk):
            for rr in range(2):
                for jj in range(NJ // 2):
                    j, r0 = c * (NJ // 2) + jj, (2 * r + rr) * MQ
                    upd.append(((slot, j, pl.ds(r0, MQ)), blk[rr][jj // 2][:, (jj % 2) * 128:(jj % 2 + 1) * 128]))
        yield from spread(_combine(
            lambda n: wide(gv[n], w2_v, n, 2, lambda c, t: b2_ref[:, pl.ds(c * DQ + t * 128, 128)]), 2, emit=emit), drain)

    def step(g, do_y, do_m):
        z = g >> 20
        lds[0] = [r.at[z] for r in full]
        last[0] = None
        del gl[:]
        k = g
        s = g - SKEW
        ky, kn, sm = k % NT, (k + 1) % NT, s % NT
        if do_m and do_y:
            qkv, w1, pr = y_qkv(), m_w1(), y_probs(k)
            _interleave((_take(qkv, 29), 29), (_take(w1, NW1), NW1))
            _interleave((_take(qkv, 29), 29), (_take(w1, NW2), NW2), (ln(kn, h_s, 8, 2), 35))
            _interleave((_take(qkv, 16), 16), (w1, 343 - NW1 - NW2), (_take(pr, NP1), NP1))
            _interleave((qkv, 13), (_take(pr, NP2), NP2))
            _interleave((m_w2(sm), 98), (_chain(pr, y_pv(k)), 130 - NP1 - NP2),
                        (_chain(v_halo(k), ln((s + 1) % NT, hn_s, 8, 2)), NVH))
            _interleave((y_wo(ky), 28), (x_out(sm), 28))
        elif do_m:
            _run(m_w1())
            _interleave((m_w2(sm), 98), (_chain(x_out(sm - 1), ln(jnp.minimum(sm + 1, NT - 1), hn_s, 8)), 60))
        else:
            qkv = y_qkv()
            pm = prep_mlp(g - 1)
            _interleave((_take(qkv, 29), 29), (_take(pm, 300), 300))
            for cp in mlp_copies(g - 1)[1::2]:
                cp.wait()
            in_copy(g + 2).wait()
            _interleave((_take(qkv, 29), 29), (_take(pm, 200), 200), (ln(kn, h_s, 8, 3, x_in(k + 2, k + 2)), 36))
            _interleave((qkv, 29), (y_probs(k, True), 64), (_take(pm, 100), 100))
            last[0] = None
            pv, wo = y_pv(k, True), y_wo(ky)
            _run(_take(pv, 16))
            _interleave((_take(wo, 4), 4), (_take(pv, 16), 16))
            _interleave((_take(wo, 4), 4), (_take(pv, 16), 16))
            _interleave((_take(wo, 12), 12), (pv, 17), (_take(pm, 104), 104))
            _interleave((wo, 8), (pm, 80))

    def prep_qkv(p, rc):
        qkv_copy(p, rc, 0).wait()
        qkv_copy(p, rc, 1).wait()
        r0 = rc * 128 if isinstance(rc, int) else pl.multiple_of(rc * 128, 128)
        top = pltpu.bitcast(wqkv_r[p, pl.ds(r0, 128), :], U32)
        bot = pltpu.bitcast(wqkv_r[p, pl.ds(KH + r0, 128), :], U32)
        wt = jnp.concatenate([top, bot], axis=0).T
        for h in range(H):
            t_s[h * PITCH:h * PITCH + DH, :] = wt[h * DH:(h + 1) * DH, :]
        d0 = rc * 64 if isinstance(rc, int) else pl.multiple_of(rc * 64, 64)
        for jj in range(NJ // 2):
            cols = [jnp.concatenate([t_s[pl.ds(4 * j + dd, H, stride=PITCH), :] for dd in range(4)], axis=0).T
                    for j in (jj, jj + NJ // 2)]
            ev, od = ([[_unpack(c[hf * 64:(hf + 1) * 64], e) for c in cols] for hf in range(2)]
                      for e in range(2))
            for i, v in enumerate(_rhs_packed(ev, od)):
                wqkv_v[p * 7 + i, pl.ds(d0, 64), jj * 128:(jj + 1) * 128] = v
            yield


    def prep_wo(z):
        for j in range(NJ):
            for h in range(H):
                if h % 8 == 0:
                    gate(wo_r, 0, D, adv=16)
                to_s[j, h % 2, (h // 2) * 24:(h // 2) * 24 + 16, :] = pltpu.bitcast(
                    wo_r[z, h * DH:(h + 1) * DH, j * 128:(j + 1) * 128], U32)
                if h % 8 == 7:
                    yield
        for jj in range(NJ // 2):
            for dp in range(8):
                for hh in range(2):
                    gate(to_s, 0, 0, 16, adv=16)
                    raw = [[[to_s[z + j, par, pl.ds(dq + hh * 8 * 24, 8, stride=24), :] for j in (jj, jj + NJ // 2)]
                            for dq in (dp, dp + 8)] for par in range(2)]
                    for e in range(2):
                        ev, od = ([[_unpack(b, e) for b in row] for row in raw[par]] for par in range(2))
                        for i, v in enumerate(_rhs_packed(ev, od)):
                            wo_v[i, pl.ds((2 * dp + e) * 16 + hh * 8, 8), jj * 128:(jj + 1) * 128] = v
                    yield

    def startup():
        in_copy(0).start()
        for p in range(3):
            if p == 2:
                in_copy(1).start()
            for rc in range(4):
                qkv_copy(p, rc, 0).start()
                qkv_copy(p, rc, 1).start()
        wo_copy().start()
        in_copy(2).start()
        for c in range(NCH):
            for cp in mlp_copies(c)[0::2] + mlp_copies(c)[1::2]:
                cp.start()
            in_copy(3 + c).start()
        for t in range(3 + NCH, NT):
            in_copy(t).start()
        hk[...] = jnp.zeros(hk.shape, F32)
        hvv[...] = jnp.zeros(hvv.shape, F32)
        in_copy(0).wait()
        _run(x_in(0, 0))
        _run(ln(0, h_s, 16))


        def prep_q(rc, carry):
            _run(prep_qkv(0, rc))
            return rc >> 20

        z = jax.lax.fori_loop(0, 4, prep_q, 0)
        lds[0] = [r.at[z] for r in full]
        qkv = y_qkv(True)
        nxt = x_in(1, 1)
        for it in range(4, 12):
            if it == 8:
                in_copy(1).wait()
            _interleave((prep_qkv(it // 4, it % 4), 4), (_take(qkv, 7), 7), (_take(nxt, 8), 8) if it >= 8 else None)
        pr = y_probs(0, True)
        _interleave((_take(qkv, 10), 10), (_take(pr, 24), 24))
        wo_copy().wait()
        _interleave((qkv, 18), (pr, 40), (prep_wo(z), 100))
        in_copy(2).wait()
        last[0] = None
        pv, wo = y_pv(0, True), y_wo(0)
        _run(_take(pv, 16))
        _interleave((_take(wo, 4), 4), (_take(pv, 16), 16))
        _interleave((_take(wo, 4), 4), (_take(pv, 16), 16))
        _interleave((wo, 20), (pv, 30), (ln(z + 1, h_s, 8, 4, x_in(2, 2)), 38))

    def p_step(g, carry):
        for cp in mlp_copies(g - 1)[0::2]:
            cp.wait()
        step(g, True, False)
        return carry

    def s_step(g, carry):
        step(g, True, True)

        @pl.when(jnp.logical_and(g >= SKEW + NT, g < NI - 1))
        def _():
            out_copy(g - SKEW - NT).start()
        return carry

    def e_step(g, carry):
        step(g, False, True)
        out_copy(g - SKEW - NT - 1).start()
        return carry

    startup()
    jax.lax.fori_loop(1, SKEW, p_step, 0)

    def load_x(t, carry):
        in_copy(t).wait()
        _run(x_in(t, t))
        return carry

    jax.lax.fori_loop(2 + SKEW, NT, load_x, 0)
    last[0] = None
    _run(ln(0, hn_s, 16))
    jax.lax.fori_loop(SKEW, NI, s_step, 0)
    jax.lax.fori_loop(NI, NI + SKEW, e_step, 0)
    last[0] = None
    _run(x_out(NT - 1))
    out_copy(NT - 1).start()
    for t in range(NT):
        out_copy(t).wait()


@jax.jit
def pallas_interleave_layers__sliding_local_dilated__dense_activation_gelu__prompt_kernel(
        A_x, A_wqkv, A_wo, B_x, B_w1, B_b1, B_w2, B_b2):
    x = A_x.reshape(S, D)
    hbm = pl.BlockSpec(memory_space=pl.ANY)
    vm = pltpu.VMEM
    out = pl.pallas_call(
        _kernel,
        in_specs=[hbm, hbm, hbm, hbm, pl.BlockSpec(memory_space=vm), hbm, pl.BlockSpec(memory_space=vm)],
        out_specs=hbm,
        out_shape=jax.ShapeDtypeStruct((S, D), BF16),
        scratch_shapes=[
            vm((NT, T, D), BF16),
            vm((NT + 2, NJ, T, 128), F32),
            vm((1, T + 8, D), F32),
            vm((1, 2 * T + 8, D), F32), vm((1, T + 8 * HALO + 8, D), F32), vm((1, T + 8 * HALO + 8, D), F32),
            vm((2, 8 * HALO, D), F32), vm((2, 8 * HALO, D), F32),
            vm((H * PITCH, 128), U32), vm((NJ, 2, 16 * 24, 128), U32),
            vm((3, D, D), BF16), vm((1, D + 16, D), BF16), vm((D + 16, F), BF16), vm((F + 16, D), BF16),
            vm((21, KH // 2, KH), U32), vm((7, KH // 2, KH), U32),
            vm((49, DQ // 2, FQ), U32), vm((49, FQ // 2, DQ), U32),
            pltpu.SemaphoreType.DMA((25 + 8 * NCH + 2 * NT,)),
        ],
        compiler_params=pltpu.CompilerParams(vmem_limit_bytes=127 * 1024 * 1024),
    )(x, A_wqkv, A_wo, B_w1, B_b1.reshape(1, F), B_w2, B_b2.reshape(1, D))
    return out.reshape(1, S, D)
```
